```python
import os as _os
_os.environ.setdefault('JAX_PLATFORMS', 'cpu')
import jax
import jax.numpy as jnp

def _softmax(x, axis=-1):
    return jax.nn.softmax(x, axis=axis)

def _gelu(x):
    return jax.nn.gelu(x, approximate=True)

def _silu(x):
    return jax.nn.silu(x)

def _sigmoid(x):
    return jax.nn.sigmoid(x)

def _layernorm(x, axis=-1, eps=1e-05):
    m = jnp.mean(x, axis=axis, keepdims=True)
    v = jnp.var(x, axis=axis, keepdims=True)
    return (x - m) / jnp.sqrt(v + eps)

def _scatter_add(tgt, idx, src, axis=0):
    return tgt.at[idx].add(src)

def _segment_sum(src, seg, n):
    return jax.ops.segment_sum(src, seg, n)

class _Rng:

    def __init__(self, key):
        self._k = key

    def _next(self):
        self._k, sub = jax.random.split(self._k)
        return sub

    def normal(self, shape):
        return jax.random.normal(self._next(), shape, dtype=jnp.bfloat16)

    def randint(self, lo, hi, shape):
        return jax.random.randint(self._next(), shape, lo, hi, dtype=jnp.int32)

    def uniform(self, shape, lo=0.0, hi=1.0):
        return jax.random.uniform(self._next(), shape, jnp.bfloat16, lo, hi)

    def permutation(self, n):
        return jax.random.permutation(self._next(), n)
kernel_name = 'gated_mix__mha_block__memory_aug_recurrent_mem_tr__prompt'

def setup_inputs():
    _rng = _Rng(jax.random.key(int.from_bytes(__import__("os").urandom(4), "little")))
    _w = lambda a: (lambda t: t.astype(jnp.bfloat16) if jnp.issubdtype(t.dtype, jnp.floating) else t)(jnp.asarray(a))

    def _A_setup():
        B, S, D, H = (1, 2048, 512, 32)
        return {'x': _w((lambda *s: _rng.normal(s) * 0.05)(B, S, D)), 'wqkv': _w((lambda *s: _rng.normal(s) * 0.8)(D, 3 * D)), 'wo': _w((lambda *s: _rng.normal(s) * 0.05)(D, D))}
    _A_in = _A_setup()

    def _B_setup():
        B, S, Dm = (1, 2048, 512)
        H, Dh = (32, 128)
        M, seg = (8, 32)
        seg = min(seg, S)
        S = S // seg * seg
        return {'x': _w((lambda *s: _rng.normal(s) * 0.05)(B, S, Dm)), 'mem0': _w((lambda *s: _rng.normal(s) * 0.8)(B, M, Dm)), 'Wq': _w((lambda *s: _rng.normal(s) * 1.6)(Dm, H, Dh) * Dm ** (-0.5)), 'Wk': _w((lambda *s: _rng.normal(s) * 1.6)(Dm, H, Dh) * Dm ** (-0.5)), 'Wv': _w((lambda *s: _rng.normal(s) * 0.8)(Dm, H, Dh) * Dm ** (-0.5)), 'Wo': _w((lambda *s: _rng.normal(s) * 0.8)(H, Dh, Dm) * (H * Dh) ** (-0.5)), 'seg_len': seg}
    _B_in = _B_setup()
    return {'A_x': _A_in['x'], 'A_wqkv': _A_in['wqkv'], 'A_wo': _A_in['wo'], 'B_x': _B_in['x'], 'B_mem0': _B_in['mem0'], 'B_Wq': _B_in['Wq'], 'B_Wk': _B_in['Wk'], 'B_Wv': _B_in['Wv'], 'B_Wo': _B_in['Wo'], 'B_seg_len': _B_in['seg_len'], 'gate_w': _w((lambda *s: _rng.normal(s) * 0.05)(512) * 16.0)}

def reference(A_x, A_wqkv, A_wo, B_x, B_mem0, B_Wq, B_Wk, B_Wv, B_Wo, B_seg_len, gate_w):

    def _A_ref(x, wqkv, wo):
        B, S, D = x.shape
        H = 32
        Dh = D // H
        qkv = (lambda x, *d: x.transpose(*d))((x @ wqkv).reshape(B, S, 3, H, Dh), 2, 0, 3, 1, 4)
        q, k, v = (qkv[0], qkv[1], qkv[2])
        scores = jnp.einsum('bhqd,bhkd->bhqk', q, k) * Dh ** (-0.5)
        p = _softmax(scores, axis=-1)
        o = jnp.einsum('bhqk,bhkd->bhqd', p, v)
        return (lambda x, *d: x.transpose(*d))(o, 0, 2, 1, 3).reshape(B, S, D) @ wo

    def _B_ref(x, mem0, Wq, Wk, Wv, Wo, seg_len):
        B, S, Dm = x.shape
        H, Dh = (Wq.shape[1], Wq.shape[2])
        M = mem0.shape[1]
        scale = Dh ** (-0.5)
        n_seg = S // seg_len
        L = M + seg_len
        idx = jnp.arange(L)
        mask = (idx[:, None] < M) | (idx[:, None] >= idx[None, :])
        mem = mem0
        outs = []
        for s in range(n_seg):
            xs = x[:, s * seg_len:(s + 1) * seg_len, :].copy()
            h = jnp.concatenate([mem, xs], axis=1)
            q = jnp.einsum('btd,dhe->bhte', h, Wq)
            k = jnp.einsum('btd,dhe->bhte', h, Wk)
            v = jnp.einsum('btd,dhe->bhte', h, Wv)
            scores = jnp.einsum('bhqe,bhke->bhqk', q, k) * scale
            scores = jnp.where(mask[None, None], scores, -1000000000.0)
            p = _softmax(scores, axis=-1)
            o = jnp.einsum('bhqk,bhke->bhqe', p, v)
            o = jnp.einsum('bhte,hed->btd', o, Wo)
            mem = o[:, :M, :].copy()
            outs.append(o[:, M:, :])
        return jnp.concatenate(outs, axis=1)
    x = A_x
    g = _sigmoid((x * gate_w).sum(-1, keepdims=True))
    a = _A_ref(x, A_wqkv, A_wo)
    b = _B_ref(x, B_mem0, B_Wq, B_Wk, B_Wv, B_Wo, B_seg_len)
    return g * a + (1 - g) * b
```

```python
import functools

import jax
import jax.numpy as jnp
from jax.experimental import pallas as pl
from jax.experimental.pallas import tpu as pltpu

F32 = jnp.float32
BF16 = jnp.bfloat16

S_LEN = 2048
D = 512
HA = 32
DHA = 16
HB = 32
DHB = 128
NMEM = 8
SEG = 32
L = NMEM + SEG
XIN = 24
XEX = SEG - XIN
NCH = XIN + NMEM
QB = 128
NQB = S_LEN // QB
SPQ = QB // SEG
GB = 4
NGB = HB // GB
GW = GB * DHB
KC = 128
NKC = S_LEN // KC
HD = HB * DHB
NQKV = 3 * HD
SCALE_B = 0.08837890625
NEG = -1000000000.0
L2 = 2 * L


def _dot(a, b):
    return jnp.dot(a, b, preferred_element_type=F32)


def _dot_nt(a, b):
    return jax.lax.dot_general(a, b, (((1,), (1,)), ((), ())), preferred_element_type=F32)


def _dot_tt(a, b):
    return jax.lax.dot_general(a, b, (((0,), (1,)), ((), ())), preferred_element_type=F32)


def _dot_tn(a, b):
    return jax.lax.dot_general(a, b, (((0,), (0,)), ((), ())), preferred_element_type=F32)


def _kernel(x_hbm, wqkv_hbm, woa_hbm, mem0_ref, wq_hbm, wk_hbm, wv_hbm, wob_hbm, gw_ref,
            o_ref,
            x_ref, wqkv_ref, woa_ref, wraw_ref, wob_ref,
            wB_scr, ka_scr, qa_scr, vat_scr, mem_scr, s_scr, mx_scr, ot_scr, b_scr, xq_scr, od_scr,
            sems):
    qb = pl.program_id(0)
    qrow0 = pl.multiple_of(qb * QB, QB)

    def build_qm4(q0, j_, half):
        qm_all = qa_scr[j_, pl.ds(q0, QB), :]
        lane = jax.lax.broadcasted_iota(jnp.int32, (QB, 128), 1)
        zero = jnp.zeros_like(qm_all)
        return jnp.concatenate(
            [jnp.where(lane // DHA == half * 4 + i, qm_all, zero) for i in range(4)], axis=0)

    def pass1_chunk(c, buf, j_, qm4, rmax):
        st = _dot_nt(ka_scr[j_, c * KC:(c + 1) * KC, :], qm4)
        s_scr[buf, c * KC:(c + 1) * KC, :] = st
        m8 = jnp.max(st.reshape(KC // 8, 8, 4 * QB), axis=0)
        return m8 if rmax is None else jnp.maximum(rmax, m8)

    def pass2_chunk(c, buf, j_, half, mx, state):
        lsum, ots = state
        new_l, new_o = [], []
        for i in range(4):
            cols = slice(i * QB, (i + 1) * QB)
            p = jnp.exp(s_scr[buf, c * KC:(c + 1) * KC, cols] - mx[:, cols])
            l8 = jnp.sum(p.reshape(KC // 8, 8, QB), axis=0)
            new_l.append(l8 if lsum is None else lsum[i] + l8)
            hrow0 = j_ * 128 + (half * 4 + i) * DHA
            d = _dot(vat_scr[c, hrow0:hrow0 + DHA, :], p.astype(BF16))
            new_o.append(d if ots is None else ots[i] + d)
        return new_l, new_o

    def pass2_finish(j_, half, state):
        lsum, ots = state
        for i in range(4):
            hrow0 = j_ * 128 + (half * 4 + i) * DHA
            l = jnp.sum(lsum[i], axis=0, keepdims=True)
            ot_scr[hrow0:hrow0 + DHA, :] = (ots[i] / l).astype(BF16)

    @pl.when(qb == 0)
    def _prologue():
      with jax.named_scope("prologue"):
        cp_x = pltpu.make_async_copy(x_hbm, x_ref, sems.at[0])
        cp_wqkv = pltpu.make_async_copy(wqkv_hbm, wqkv_ref, sems.at[1])
        cp_woa = pltpu.make_async_copy(woa_hbm, woa_ref, sems.at[2])
        cp_w = [pltpu.make_async_copy(src, wraw_ref.at[i], sems.at[3 + i])
                for i, src in enumerate((wq_hbm, wk_hbm, wv_hbm))]
        cp_wob = [pltpu.make_async_copy(wob_hbm.at[:, n * 128:(n + 1) * 128], wob_ref.at[n], sems.at[6 + n])
                  for n in range(4)]
        cp_x.start()
        cp_wqkv.start()
        cp_x.wait()
        cp_wqkv.wait()
        cp_w[0].start()
        NB = 8
        RB = S_LEN // NB
        WB = D // NB

        def relayout(i, which):
            r0 = pl.multiple_of(i * WB, WB)
            w2 = wraw_ref[which, pl.ds(r0, WB)].reshape(WB, HD)
            for n in range(HB):
                wB_scr[which * HB + n, pl.ds(r0, WB), :] = w2[:, n * DHB:(n + 1) * DHB]

        def q_body(i, carry):
            r0 = pl.multiple_of(i * RB, RB)
            q = _dot(x_ref[pl.ds(r0, RB), :], wqkv_ref[:, 0:D]).astype(BF16)
            q = (q.astype(F32) * 0.25).astype(BF16)
            for jj in range(4):
                qa_scr[jj, pl.ds(r0, RB), :] = q[:, jj * 128:(jj + 1) * 128]
            return carry

        jax.lax.fori_loop(0, NB, q_body, 0)
        cp_w[0].wait()
        cp_w[1].start()

        def k_body(i, carry):
            r0 = pl.multiple_of(i * RB, RB)
            k = _dot(x_ref[pl.ds(r0, RB), :], wqkv_ref[:, D:2 * D]).astype(BF16)
            for jj in range(4):
                ka_scr[jj, pl.ds(r0, RB), :] = k[:, jj * 128:(jj + 1) * 128]
            relayout(i, 0)
            return carry

        jax.lax.fori_loop(0, NB, k_body, 0)
        cp_w[1].wait()
        cp_w[2].start()

        def v_body(i, carry):
            for u in range(RB // KC):
                r0 = pl.multiple_of(i * RB + u * KC, KC)
                vat_scr[i * (RB // KC) + u] = _dot_tt(wqkv_ref[:, 2 * D:3 * D], x_ref[pl.ds(r0, KC), :]).astype(BF16)
            relayout(i, 1)
            return carry

        jax.lax.fori_loop(0, NB, v_body, 0)
        cp_w[2].wait()
        for cp in cp_wob:
            cp.start()
        cp_woa.start()
        mem_scr[...] = mem0_ref[...]
        qm4 = build_qm4(0, 0, 0)

        def s_body(i, rmax):
            for u in range(NKC // NB):
                r0 = pl.multiple_of((i * (NKC // NB) + u) * KC, KC)
                st = _dot_nt(ka_scr[0, pl.ds(r0, KC), :], qm4)
                s_scr[0, pl.ds(r0, KC), :] = st
                rmax = jnp.maximum(rmax, jnp.max(st.reshape(KC // 8, 8, 4 * QB), axis=0))
            relayout(i, 2)
            return rmax

        rmax = jax.lax.fori_loop(0, NB, s_body, jnp.full((8, 4 * QB), -jnp.inf, F32))
        mx_scr[...] = jnp.max(rmax, axis=0, keepdims=True)
        for cp in cp_wob:
            cp.wait()
        cp_woa.wait()

    rho = jax.lax.broadcasted_iota(jnp.int32, (L2, L2), 0)
    gam = jax.lax.broadcasted_iota(jnp.int32, (L2, L2), 1)

    def _head(t):
        return ((t >= NCH) & (t < 2 * NCH)) | (t >= 2 * NCH + XEX)

    def _local(t):
        return jnp.where(t < 2 * NCH, t % NCH, NCH + (t - 2 * NCH) % XEX)

    lr, lc = _local(rho), _local(gam)
    allowed = (_head(rho) == _head(gam)) & (
        ((lr >= XIN) & (lr < NCH)) | ((lc >= XIN) & (lc < NCH)) | (lc <= lr))

    qbn0 = pl.multiple_of(((qb + 1) % NQB) * QB, QB)
    mx_cur = mx_scr[...]
    mem = mem_scr[...]

    for j in range(SPQ):
        seg0 = qrow0 + j * SEG
        if j == 0:
            h = jnp.concatenate(
                [x_ref[pl.ds(seg0, XIN), :], mem]
                + [x_ref[pl.ds(qrow0 + i * SEG + XIN, XEX), :] for i in range(SPQ)], axis=0)
        else:
            h = jnp.concatenate([x_ref[pl.ds(seg0, XIN), :], mem], axis=0)

        def b_proj(which, g, h=h, j=j):
            cols = slice(which * HD + g * GW, which * HD + (g + 1) * GW)
            y = jnp.concatenate([_dot(h, wB_scr[which * HB + g * GB + hh]) for hh in range(GB)], axis=1)
            if j == 0:
                xq_scr[:, :, cols] = y[NCH + XEX:].reshape(SPQ - 1, XEX, GW)
                return y[0:NCH], y[NCH:NCH + XEX]
            return y, xq_scr[j - 1, :, cols]

        def stack2(y, ex, pr):
            a, b = slice(2 * pr * DHB, (2 * pr + 1) * DHB), slice((2 * pr + 1) * DHB, (2 * pr + 2) * DHB)
            return jnp.concatenate([y[:, a], y[:, b], ex[:, a], ex[:, b]], axis=0).astype(BF16)

        def b_qkv(g):
            yq, yk, yv = b_proj(0, g), b_proj(1, g), b_proj(2, g)
            return [[stack2(y, ex, pr) for pr in range(2)] for (y, ex) in (yq, yk, yv)]

        def b_scores(q2, k2):
            return [_dot_nt(q2[pr], k2[pr]) for pr in range(2)]

        def b_softmax(scs):
            ps, ls = [], []
            for sc in scs:
                sc = jnp.where(allowed, sc * SCALE_B, NEG)
                m = jnp.max(sc, axis=1, keepdims=True)
                p = jnp.exp(sc - m)
                ls.append(jnp.sum(p, axis=1, keepdims=True))
                ps.append(p.astype(BF16))
            return ps, ls

        def b_pv(ps, v2):
            return [_dot(ps[pr], v2[pr]) for pr in range(2)]

        def b_out(g, os_, ls, acc, j=j):
            o = [(o / l).astype(BF16) for o, l in zip(os_, ls)]
            og = jnp.concatenate([o[0][0:NCH], o[0][NCH:2 * NCH], o[1][0:NCH], o[1][NCH:2 * NCH]], axis=1)
            od = jnp.concatenate([o[0][2 * NCH:2 * NCH + XEX], o[0][2 * NCH + XEX:L2],
                                  o[1][2 * NCH:2 * NCH + XEX], o[1][2 * NCH + XEX:L2]], axis=1)
            cols = slice(g * GW, (g + 1) * GW)
            if j < SPQ - 1:
                od_scr[j, :, cols] = od.astype(F32)
                lhs = og
            else:
                odp = od_scr[:, :, cols].reshape((SPQ - 1) * XEX, GW)
                lhs = jnp.concatenate([og.astype(F32), odp, od.astype(F32)], axis=0).astype(BF16)
            d = jnp.concatenate([_dot(lhs, wob_ref[n, cols, :]) for n in range(4)], axis=1)
            return d if acc is None else acc + d

        acc = None
        for ph in range(2):
            if ph == 0:
                qm4, jw = build_qm4(qrow0, j, 1), j
            elif j < SPQ - 1:
                qm4, jw = build_qm4(qrow0, j + 1, 0), j + 1
            else:
                qm4, jw = build_qm4(qbn0, 0, 0), 0
            a_state = dict(rmax=None, st=(None, None))

            def a_p1(c, ph=ph, jw=jw, qm4=qm4, a_state=a_state):
                a_state['rmax'] = pass1_chunk(c, 1 - ph, jw, qm4, a_state['rmax'])

            def a_p2(c, ph=ph, j=j, a_state=a_state, mx=mx_cur):
                a_state['st'] = pass2_chunk(c, ph, j, ph, mx, a_state['st'])

            for gi in range(NGB // 2):
                g = ph * (NGB // 2) + gi
                c0 = 4 * gi
                yq = b_proj(0, g)
                a_p2(c0)
                yk = b_proj(1, g)
                a_p2(c0 + 1)
                yv = b_proj(2, g)
                a_p2(c0 + 2)
                q2, k2, v2 = [[stack2(y, ex, pr) for pr in range(2)] for (y, ex) in (yq, yk, yv)]
                scs = b_scores(q2, k2)
                a_p1(c0)
                ps, ls = b_softmax(scs)
                a_p1(c0 + 1)
                os_ = b_pv(ps, v2)
                a_p1(c0 + 2)
                acc = b_out(g, os_, ls, acc)
                a_p1(c0 + 3)
                a_p2(c0 + 3)
            mx_cur = jnp.max(a_state['rmax'], axis=0, keepdims=True)
            pass2_finish(j, ph, a_state['st'])

        outb = acc.astype(BF16)
        mem = outb[XIN:NCH]
        b_scr[j * SEG:j * SEG + XIN, :] = outb[0:XIN].astype(F32)
        if j == SPQ - 1:
            for i in range(SPQ):
                b_scr[i * SEG + XIN:(i + 1) * SEG, :] = outb[NCH + i * XEX:NCH + (i + 1) * XEX].astype(F32)

    mx_scr[...] = mx_cur
    mem_scr[...] = mem

    a = _dot_tn(ot_scr[...], woa_ref[...]).astype(BF16).astype(F32)
    xb = x_ref[pl.ds(qrow0, QB), :].astype(F32)
    prod = (xb * gw_ref[...].astype(F32)).astype(BF16).astype(F32)
    gsum = jnp.sum(prod, axis=1, keepdims=True).astype(BF16).astype(F32)
    g = jax.nn.sigmoid(gsum).astype(BF16).astype(F32)
    ga = (g * a).astype(BF16).astype(F32)
    omg = (1.0 - g).astype(BF16).astype(F32)
    gb = (omg * b_scr[...]).astype(BF16).astype(F32)
    o_ref[...] = (ga + gb).astype(o_ref.dtype)


@functools.partial(jax.jit, static_argnames=("B_seg_len",))
def pallas_gated_mix__mha_block__memory_aug_recurrent_mem_tr__prompt_kernel(
    A_x, A_wqkv, A_wo, B_x, B_mem0, B_Wq, B_Wk, B_Wv, B_Wo, B_seg_len, gate_w):
    del B_x
    assert B_seg_len == SEG
    assert A_x.shape == (1, S_LEN, D) and B_mem0.shape == (1, NMEM, D)
    x = A_x.reshape(S_LEN, D)
    mem0 = B_mem0.reshape(NMEM, D)
    wob = B_Wo.reshape(HD, D)
    gw = gate_w.reshape(1, D)

    hbm = pl.BlockSpec(memory_space=pl.ANY)

    def whole(shape):
        return pl.BlockSpec(shape, lambda s: (0,) * len(shape))

    out = pl.pallas_call(
        _kernel,
        grid=(NQB,),
        in_specs=[hbm, hbm, hbm, whole((NMEM, D)), hbm, hbm, hbm, hbm, whole((1, D))],
        out_specs=pl.BlockSpec((QB, D), lambda s: (s, 0)),
        out_shape=jax.ShapeDtypeStruct((S_LEN, D), BF16),
        scratch_shapes=[
            pltpu.VMEM((S_LEN, D), BF16),
            pltpu.VMEM((D, 3 * D), BF16),
            pltpu.VMEM((D, D), BF16),
            pltpu.VMEM((3, D, HB, DHB), BF16),
            pltpu.VMEM((4, HD, 128), BF16),
            pltpu.VMEM((3 * HB, D, DHB), BF16),
            pltpu.VMEM((4, S_LEN, 128), BF16),
            pltpu.VMEM((4, S_LEN, 128), BF16),
            pltpu.VMEM((NKC, D, KC), BF16),
            pltpu.VMEM((NMEM, D), BF16),
            pltpu.VMEM((2, S_LEN, 4 * QB), F32),
            pltpu.VMEM((1, 4 * QB), F32),
            pltpu.VMEM((D, QB), BF16),
            pltpu.VMEM((QB, D), F32),
            pltpu.VMEM((SPQ - 1, XEX, NQKV), F32),
            pltpu.VMEM((SPQ - 1, XEX, HD), F32),
            pltpu.SemaphoreType.DMA((10,)),
        ],
        compiler_params=pltpu.CompilerParams(
            dimension_semantics=("arbitrary",),
            vmem_limit_bytes=110 * 1024 * 1024,
        ),
    )(x, A_wqkv, A_wo, mem0, B_Wq, B_Wk, B_Wv, wob, gw)
    return out.reshape(1, S_LEN, D)
```

```python
import functools

import jax
import jax.numpy as jnp
from jax.experimental import pallas as pl
from jax.experimental.pallas import tpu as pltpu

F32 = jnp.float32
BF16 = jnp.bfloat16

S_LEN = 2048
D = 512
HA = 32
DHA = 16
HB = 32
DHB = 128
NMEM = 8
SEG = 32
L = NMEM + SEG
XIN = 24
XEX = SEG - XIN
NCH = XIN + NMEM
QB = 128
NQB = S_LEN // QB
SPQ = QB // SEG
GB = 4
NGB = HB // GB
GW = GB * DHB
HG = 8
KC = 128
NKC = S_LEN // KC
KC1 = 64
NKC1 = S_LEN // KC1
HD = HB * DHB
NQKV = 3 * HD
SCALE_B = 0.08837890625
NEG = -1000000000.0
L2 = 2 * L
ORDER = 'Q p2 K V p1 S p2 SM p1 p2 PV p1 OUT p1 p2'.split()


def _dot(a, b):
    return jnp.dot(a, b, preferred_element_type=F32)


def _dot_nt(a, b):
    return jax.lax.dot_general(a, b, (((1,), (1,)), ((), ())), preferred_element_type=F32)


def _dot_tn(a, b):
    return jax.lax.dot_general(a, b, (((0,), (0,)), ((), ())), preferred_element_type=F32)


def _kernel(x_hbm, wqkv_hbm, woa_hbm, mem0_ref, wq_hbm, wk_hbm, wv_hbm, wob_hbm, gw_ref,
            o_ref,
            x_ref, wqkv_ref, woa_ref, wraw_ref, wob_ref,
            wB_scr, wat_scr, ka_scr, qt_scr, vat_scr, mem_scr, s_scr, mx_scr, ot_scr, b_scr, a_scr, xq_scr, od_scr,
            sems):
    qb = pl.program_id(0)
    qrow0 = pl.multiple_of(qb * QB, QB)

    def build_qm8(q0, j_):
        qt = qt_scr[j_, :, pl.ds(q0, QB)]
        sub = jax.lax.broadcasted_iota(jnp.int32, (128, QB), 0) // DHA
        zero = jnp.zeros_like(qt)
        return jnp.concatenate([jnp.where(sub == i, qt, zero) for i in range(HG)], axis=1)

    def pass1_chunk(r0, buf, j_, qm8, rmax):
        st = _dot(ka_scr[j_, pl.ds(r0, KC1), :], qm8)
        s_scr[buf, pl.ds(r0, KC1), :] = st
        m8 = jnp.max(st.reshape(KC1 // 8, 8, HG * QB), axis=0)
        return m8 if rmax is None else jnp.maximum(rmax, m8)

    ones_blk = jnp.where(jax.lax.broadcasted_iota(jnp.int32, (DHA, KC), 0) == 0, 1.0, 0.0).astype(BF16)

    def pass2_chunk(c, half, buf, j_, mx, state):
        new = []
        for i in range(4):
            hh = half * 4 + i
            cols = slice(hh * QB, (hh + 1) * QB)
            p = jnp.exp(s_scr[buf, c * KC:(c + 1) * KC, cols] - mx[:, cols])
            hrow0 = j_ * 128 + hh * DHA
            lhs = jnp.concatenate([vat_scr[c, hrow0:hrow0 + DHA, :], ones_blk], axis=0)
            d = _dot(lhs, p.astype(BF16))
            new.append(d if state is None else state[i] + d)
        return new

    def pass2_finish(j_, half, state):
        for i in range(4):
            hrow0 = j_ * 128 + (half * 4 + i) * DHA
            ot_scr[hrow0:hrow0 + DHA, :] = (state[i][0:DHA] / state[i][DHA:DHA + 1]).astype(BF16)

    def a_part(g_):
        rows = slice(g_ * 128, (g_ + 1) * 128)
        return _dot_tn(ot_scr[rows, :], woa_ref[rows, :])

    @pl.when(qb == 0)
    def _prologue():
        NB = 8
        RB = S_LEN // NB
        WB = D // NB
        WP = WB // 4
        cp_wqkv = pltpu.make_async_copy(wqkv_hbm, wqkv_ref, sems.at[0])
        cp_x = [pltpu.make_async_copy(x_hbm.at[pl.ds(i * RB, RB)], x_ref.at[pl.ds(i * RB, RB)], sems.at[10 + i])
                for i in range(NB)]
        cp_woa = pltpu.make_async_copy(woa_hbm, woa_ref, sems.at[2])
        cp_w = [pltpu.make_async_copy(src, wraw_ref.at[i], sems.at[3 + i])
                for i, src in enumerate((wq_hbm, wk_hbm, wv_hbm))]
        cp_wob = [pltpu.make_async_copy(wob_hbm.at[:, n * 128:(n + 1) * 128], wob_ref.at[n], sems.at[6 + n])
                  for n in range(4)]
        cp_wqkv.start()
        for cp in cp_x:
            cp.start()
        cp_w[0].start()
        cp_wqkv.wait()
        wat_scr[0:D, :] = wqkv_ref[:, 0:D].T
        wat_scr[D:2 * D, :] = wqkv_ref[:, 2 * D:3 * D].T

        def relayout(i, u, which):
            r0 = pl.multiple_of(i * WB + u * WP, WP)
            wB_scr[pl.ds(which * HB, HB), pl.ds(r0, WP), :] = jnp.swapaxes(wraw_ref[which, pl.ds(r0, WP)], 0, 1)

        def k_body(i, carry):
            r0 = pl.multiple_of(i * RB, RB)
            pltpu.make_async_copy(x_hbm.at[pl.ds(r0, RB)], x_ref.at[pl.ds(r0, RB)], sems.at[10 + i]).wait()
            k = _dot(x_ref[pl.ds(r0, RB), :], wqkv_ref[:, D:2 * D]).astype(BF16)
            for jj in range(4):
                ka_scr[jj, pl.ds(r0, RB), :] = k[:, jj * 128:(jj + 1) * 128]
            return carry

        jax.lax.fori_loop(0, NB, k_body, 0, unroll=2)
        cp_w[0].wait()
        cp_w[1].start()

        def qv_body(cc, which):
            r0 = pl.multiple_of(cc * KC, KC)
            xc = x_ref[pl.ds(r0, KC), :]
            for u in range(4):
                relayout(cc % NB, u, which)
                piece = _dot_nt(wat_scr[u * 256:(u + 1) * 256, :], xc).astype(BF16)
                if u < 2:
                    qt = (piece.astype(F32) * 0.25).astype(BF16)
                    for v in range(2):
                        qt_scr[2 * u + v, :, pl.ds(r0, KC)] = qt[v * 128:(v + 1) * 128]
                else:
                    vat_scr[cc, (u - 2) * 256:(u - 1) * 256, :] = piece
            return which

        jax.lax.fori_loop(0, NB, qv_body, 0, unroll=2)
        cp_w[1].wait()
        cp_w[2].start()
        jax.lax.fori_loop(NB, 2 * NB, qv_body, 1, unroll=2)
        cp_w[2].wait()
        for cp in cp_wob:
            cp.start()
        cp_woa.start()
        mem_scr[...] = mem0_ref[...]
        qm8 = build_qm8(0, 0)

        def s_body(i, rmax):
            for u in range(NKC1 // NB):
                relayout(i, u, 2)
                rmax = pass1_chunk(pl.multiple_of((i * (NKC1 // NB) + u) * KC1, KC1), 0, 0, qm8, rmax)
            return rmax

        rmax = jax.lax.fori_loop(0, NB, s_body, jnp.full((8, HG * QB), -jnp.inf, F32), unroll=2)
        mx_scr[...] = jnp.max(rmax, axis=0, keepdims=True)
        for cp in cp_wob:
            cp.wait()
        cp_woa.wait()

    rho = jax.lax.broadcasted_iota(jnp.int32, (L2, L2), 0)
    gam = jax.lax.broadcasted_iota(jnp.int32, (L2, L2), 1)

    def _head(t):
        return ((t >= NCH) & (t < 2 * NCH)) | (t >= 2 * NCH + XEX)

    def _local(t):
        return jnp.where(t < 2 * NCH, t % NCH, NCH + (t - 2 * NCH) % XEX)

    lr, lc = _local(rho), _local(gam)
    allowed = (_head(rho) == _head(gam)) & (
        ((lr >= XIN) & (lr < NCH)) | ((lc >= XIN) & (lc < NCH)) | (lc <= lr))

    qbn0 = pl.multiple_of(((qb + 1) % NQB) * QB, QB)
    mx_cur = mx_scr[...]
    mem = mem_scr[...]

    for j in range(SPQ):
        seg0 = qrow0 + j * SEG
        if j == 0:
            h = jnp.concatenate(
                [x_ref[pl.ds(seg0, XIN), :], mem]
                + [x_ref[pl.ds(qrow0 + i * SEG + XIN, XEX), :] for i in range(SPQ)], axis=0)
        else:
            h = jnp.concatenate([x_ref[pl.ds(seg0, XIN), :], mem], axis=0)

        def b_proj(which, g, h=h, j=j):
            cols = slice(which * HD + g * GW, which * HD + (g + 1) * GW)
            y = jnp.concatenate([_dot(h, wB_scr[which * HB + g * GB + hh]) for hh in range(GB)], axis=1)
            if j == 0:
                xq_scr[:, :, cols] = y[NCH + XEX:].reshape(SPQ - 1, XEX, GW)
                return y[0:NCH], y[NCH:NCH + XEX]
            return y, xq_scr[j - 1, :, cols]

        def stack2(y, ex, pr):
            a, b = slice(2 * pr * DHB, (2 * pr + 1) * DHB), slice((2 * pr + 1) * DHB, (2 * pr + 2) * DHB)
            return jnp.concatenate([y[:, a], y[:, b], ex[:, a], ex[:, b]], axis=0).astype(BF16)

        def b_scores(q2, k2):
            return [_dot_nt(q2[pr], k2[pr]) for pr in range(2)]

        def b_softmax(scs):
            ps, ls = [], []
            for sc in scs:
                sc = jnp.where(allowed, sc * SCALE_B, NEG)
                m = jnp.max(sc, axis=1, keepdims=True)
                p = jnp.exp(sc - m)
                ls.append(jnp.sum(p, axis=1, keepdims=True))
                ps.append(p.astype(BF16))
            return ps, ls

        def b_pv(ps, v2):
            return [_dot(ps[pr], v2[pr]) for pr in range(2)]

        def b_out(g, os_, ls, acc, j=j):
            o = [(o / l).astype(BF16) for o, l in zip(os_, ls)]
            og = jnp.concatenate([o[0][0:NCH], o[0][NCH:2 * NCH], o[1][0:NCH], o[1][NCH:2 * NCH]], axis=1)
            od = jnp.concatenate([o[0][2 * NCH:2 * NCH + XEX], o[0][2 * NCH + XEX:L2],
                                  o[1][2 * NCH:2 * NCH + XEX], o[1][2 * NCH + XEX:L2]], axis=1)
            cols = slice(g * GW, (g + 1) * GW)
            if j < SPQ - 1:
                od_scr[j, :, cols] = od.astype(F32)
                lhs = og
            else:
                odp = od_scr[:, :, cols].reshape((SPQ - 1) * XEX, GW)
                lhs = jnp.concatenate([og.astype(F32), odp, od.astype(F32)], axis=0).astype(BF16)
            d = jnp.concatenate([_dot(lhs, wob_ref[n, cols, :]) for n in range(4)], axis=1)
            return d if acc is None else acc + d

        buf = j % 2
        if j < SPQ - 1:
            qm8, jn = build_qm8(qrow0, j + 1), j + 1
        else:
            qm8, jn = build_qm8(qbn0, 0), 0
        a_state = dict(rmax=None, st=None)

        def a_p1(t, buf=buf, jn=jn, qm8=qm8, a_state=a_state):
            a_state['rmax'] = pass1_chunk(t * KC1, 1 - buf, jn, qm8, a_state['rmax'])

        def a_p2(t, buf=buf, j=j, a_state=a_state, mx=mx_cur):
            half, c = t // NKC, t % NKC
            a_state['st'] = pass2_chunk(c, half, buf, j, mx, a_state['st'])
            if c == NKC - 1:
                pass2_finish(j, half, a_state['st'])
                a_state['st'] = None

        acc = None
        n1 = n2 = 0
        for g in range(NGB):
            v_ = {}
            for act in ORDER:
                if act == 'Q':
                    v_['yq'] = b_proj(0, g)
                elif act == 'K':
                    v_['yk'] = b_proj(1, g)
                elif act == 'V':
                    v_['yv'] = b_proj(2, g)
                elif act == 'S':
                    q2, k2 = [[stack2(y, ex, pr) for pr in range(2)] for (y, ex) in (v_['yq'], v_['yk'])]
                    v_['scs'] = b_scores(q2, k2)
                elif act == 'SM':
                    v_['ps'], v_['ls'] = b_softmax(v_['scs'])
                elif act == 'PV':
                    v2 = [stack2(v_['yv'][0], v_['yv'][1], pr) for pr in range(2)]
                    v_['os'] = b_pv(v_['ps'], v2)
                elif act == 'OUT':
                    acc = b_out(g, v_['os'], v_['ls'], acc)
                elif act == 'p1':
                    a_p1(n1)
                    n1 += 1
                elif act == 'p2':
                    a_p2(n2)
                    n2 += 1
            if g == 0 and j >= 1:
                if j == 1:
                    a_scr[...] = a_part(0)
                else:
                    a_scr[...] = a_scr[...] + a_part(j - 1)
        assert n1 == NKC1 and n2 == 2 * NKC
        mx_cur = jnp.max(a_state['rmax'], axis=0, keepdims=True)

        outb = acc.astype(BF16)
        mem = outb[XIN:NCH]
        b_scr[j * SEG:j * SEG + XIN, :] = outb[0:XIN].astype(F32)
        if j == SPQ - 1:
            for i in range(SPQ):
                b_scr[i * SEG + XIN:(i + 1) * SEG, :] = outb[NCH + i * XEX:NCH + (i + 1) * XEX].astype(F32)

    mx_scr[...] = mx_cur
    mem_scr[...] = mem

    a = (a_scr[...] + a_part(SPQ - 1)).astype(BF16).astype(F32)
    xb = x_ref[pl.ds(qrow0, QB), :].astype(F32)
    prod = (xb * gw_ref[...].astype(F32)).astype(BF16).astype(F32)
    gsum = jnp.sum(prod, axis=1, keepdims=True).astype(BF16).astype(F32)
    g = jax.nn.sigmoid(gsum).astype(BF16).astype(F32)
    ga = (g * a).astype(BF16).astype(F32)
    omg = (1.0 - g).astype(BF16).astype(F32)
    gb = (omg * b_scr[...]).astype(BF16).astype(F32)
    o_ref[...] = (ga + gb).astype(o_ref.dtype)


@functools.partial(jax.jit, static_argnames=("B_seg_len",))
def pallas_gated_mix__mha_block__memory_aug_recurrent_mem_tr__prompt_kernel(
    A_x, A_wqkv, A_wo, B_x, B_mem0, B_Wq, B_Wk, B_Wv, B_Wo, B_seg_len, gate_w):
    del B_x
    assert B_seg_len == SEG
    assert A_x.shape == (1, S_LEN, D) and B_mem0.shape == (1, NMEM, D)
    x = A_x.reshape(S_LEN, D)
    mem0 = B_mem0.reshape(NMEM, D)
    wob = B_Wo.reshape(HD, D)
    gw = gate_w.reshape(1, D)

    hbm = pl.BlockSpec(memory_space=pl.ANY)

    def whole(shape):
        return pl.BlockSpec(shape, lambda s: (0,) * len(shape))

    out = pl.pallas_call(
        _kernel,
        grid=(NQB,),
        in_specs=[hbm, hbm, hbm, whole((NMEM, D)), hbm, hbm, hbm, hbm, whole((1, D))],
        out_specs=pl.BlockSpec((QB, D), lambda s: (s, 0)),
        out_shape=jax.ShapeDtypeStruct((S_LEN, D), BF16),
        scratch_shapes=[
            pltpu.VMEM((S_LEN, D), BF16),
            pltpu.VMEM((D, 3 * D), BF16),
            pltpu.VMEM((D, D), BF16),
            pltpu.VMEM((3, D, HB, DHB), BF16),
            pltpu.VMEM((4, HD, 128), BF16),
            pltpu.VMEM((3 * HB, D, DHB), BF16),
            pltpu.VMEM((2 * D, D), BF16),
            pltpu.VMEM((4, S_LEN, 128), BF16),
            pltpu.VMEM((4, 128, S_LEN), BF16),
            pltpu.VMEM((NKC, D, KC), BF16),
            pltpu.VMEM((NMEM, D), BF16),
            pltpu.VMEM((2, S_LEN, HG * QB), F32),
            pltpu.VMEM((1, HG * QB), F32),
            pltpu.VMEM((D, QB), BF16),
            pltpu.VMEM((QB, D), F32),
            pltpu.VMEM((QB, D), F32),
            pltpu.VMEM((SPQ - 1, XEX, NQKV), F32),
            pltpu.VMEM((SPQ - 1, XEX, HD), F32),
            pltpu.SemaphoreType.DMA((18,)),
        ],
        compiler_params=pltpu.CompilerParams(
            dimension_semantics=("arbitrary",),
            vmem_limit_bytes=110 * 1024 * 1024,
        ),
    )(x, A_wqkv, A_wo, mem0, B_Wq, B_Wk, B_Wv, wob, gw)
    return out.reshape(1, S_LEN, D)
```
